```python
import jax
import jax.numpy as jnp

def _softmax(x, axis=-1):
    return jax.nn.softmax(x, axis=axis)

def _gelu(x):
    return jax.nn.gelu(x, approximate=True)

def _silu(x):
    return jax.nn.silu(x)

def _sigmoid(x):
    return jax.nn.sigmoid(x)

def _layernorm(x, axis=-1, eps=1e-05):
    m = jnp.mean(x, axis=axis, keepdims=True)
    v = jnp.var(x, axis=axis, keepdims=True)
    return (x - m) / jnp.sqrt(v + eps)

def _scatter_add(tgt, idx, src, axis=0):
    return tgt.at[idx].add(src)

def _segment_sum(src, seg, n):
    return jax.ops.segment_sum(src, seg, n)

class _Rng:

    def __init__(self, key):
        self._k = key

    def _next(self):
        self._k, sub = jax.random.split(self._k)
        return sub

    def normal(self, shape):
        return jax.random.normal(self._next(), shape, dtype=jnp.bfloat16)

    def randint(self, lo, hi, shape):
        return jax.random.randint(self._next(), shape, lo, hi, dtype=jnp.int32)

    def uniform(self, shape, lo=0.0, hi=1.0):
        return jax.random.uniform(self._next(), shape, jnp.bfloat16, lo, hi)

    def permutation(self, n):
        return jax.random.permutation(self._next(), n)
kernel_name = 'adaLN_cond__compressed_kv_cla__glu_gated_geglu__decode'

def setup_inputs():
    _rng = _Rng(jax.random.key(int.from_bytes(__import__("os").urandom(4), "little")))
    _w = lambda a: (lambda t: t.astype(jnp.bfloat16) if jnp.issubdtype(t.dtype, jnp.floating) else t)(jnp.asarray(a))

    def _A_setup():
        B, H, Sq, Sk, D, M = (1, 32, 1, 32768, 128, 512)
        Dc = 4 * D
        return {'x': _w((lambda *s: _rng.normal(s) * 0.05)(B, Sq, M)), 'c_kv': _w((lambda *s: _rng.normal(s) * 0.05)(B, Sk, Dc)), 'w_q': _w((lambda *s: _rng.normal(s) * 0.05)(M, H, D) * M ** (-0.5)), 'w_uk': _w((lambda *s: _rng.normal(s) * 0.05)(Dc, H, D) * Dc ** (-0.5)), 'w_uv': _w((lambda *s: _rng.normal(s) * 0.05)(Dc, H, D) * Dc ** (-0.5)), 'w_o': _w((lambda *s: _rng.normal(s) * 0.05)(H, D, M) * (H * D) ** (-0.5))}
    _A_in = _A_setup()

    def _B_setup():
        B, S, Dm, Df = (1, 1, 512, 1792)
        return {'x': _w((lambda *s: _rng.normal(s) * 0.05)(B, S, Dm)), 'w_gate': _w((lambda *s: _rng.normal(s) * 0.05)(Dm, Df) * Dm ** (-0.5)), 'w_up': _w((lambda *s: _rng.normal(s) * 0.05)(Dm, Df) * Dm ** (-0.5)), 'w_down': _w((lambda *s: _rng.normal(s) * 0.05)(Df, Dm) * Df ** (-0.5))}
    _B_in = _B_setup()
    return {'A_x': _A_in['x'], 'A_c_kv': _A_in['c_kv'], 'A_w_q': _A_in['w_q'], 'A_w_uk': _A_in['w_uk'], 'A_w_uv': _A_in['w_uv'], 'A_w_o': _A_in['w_o'], 'B_x': _B_in['x'], 'B_w_gate': _B_in['w_gate'], 'B_w_up': _B_in['w_up'], 'B_w_down': _B_in['w_down'], 'c': _w((lambda *s: _rng.normal(s) * 0.05)(1, 512)), 'w_mod': _w((lambda *s: _rng.normal(s) * 0.05)(512, 6 * 512) * 512 ** (-0.5))}

def reference(A_x, A_c_kv, A_w_q, A_w_uk, A_w_uv, A_w_o, B_x, B_w_gate, B_w_up, B_w_down, c, w_mod):

    def _A_ref(x, c_kv, w_q, w_uk, w_uv, w_o):
        B, Sq, M = (x.shape[0], x.shape[1], x.shape[2])
        Sk = c_kv.shape[1]
        H, D = (w_q.shape[1], w_q.shape[2])
        q = jnp.einsum('bqm,mhd->bhqd', x, w_q)
        k = jnp.einsum('bkc,chd->bhkd', c_kv, w_uk)
        v = jnp.einsum('bkc,chd->bhkd', c_kv, w_uv)
        scores = jnp.einsum('bhqd,bhkd->bhqk', q, k) * D ** (-0.5)
        off = Sk - Sq
        qi = jnp.arange(Sq)[:, None]
        kj = jnp.arange(Sk)[None, :]
        cmask = kj <= qi + off
        scores = jnp.where(cmask[None, None], scores, -1000000000.0)
        p = _softmax(scores, axis=-1)
        ctx = jnp.einsum('bhqk,bhkd->bhqd', p, v)
        return jnp.einsum('bhqd,hdm->bqm', ctx, w_o)

    def _B_ref(x, w_gate, w_up, w_down):
        g = jnp.einsum('bsd,df->bsf', x, w_gate)
        u = jnp.einsum('bsd,df->bsf', x, w_up)
        h = _gelu(g) * u
        return jnp.einsum('bsf,fd->bsd', h, w_down)
    x = A_x
    mod = (_silu(c) @ w_mod).reshape(c.shape[0], 6, 1, -1)
    sa, ca, ga, sb, cb, gb = (mod[:, 0].copy(), mod[:, 1].copy(), mod[:, 2].copy(), mod[:, 3].copy(), mod[:, 4].copy(), mod[:, 5].copy())
    h = _layernorm(x, axis=-1) * (1 + ca) + sa
    x = x + ga * _A_ref(h, A_c_kv, A_w_q, A_w_uk, A_w_uv, A_w_o)
    h = _layernorm(x, axis=-1) * (1 + cb) + sb
    x = x + gb * _B_ref(h, B_w_gate, B_w_up, B_w_down)
    return x
```

```python
import functools

import jax
import jax.numpy as jnp
from jax import lax
import jax.experimental.pallas as pl
import jax.experimental.pallas.tpu as pltpu

_H = 32
_D = 128
_M = 512
_F = 1792
_SK = 32768
_T = 4096
_NCHUNK = _SK // _T
_BLK = 128
_ROWS = _BLK * _H
_NBLK = _M // _BLK
_WD_SPLITS = (0, 1024, 1536, 1792)
_EPS = 1e-5
_NT = (((1,), (1,)), ((), ()))


def _layernorm(x):
    mean = jnp.mean(x, axis=-1, keepdims=True)
    xc = x - mean
    var = jnp.mean(xc * xc, axis=-1, keepdims=True)
    return xc / jnp.sqrt(var + _EPS)


def _gelu_tanh(x):
    k = 0.7978845608028654
    return 0.5 * x * (1.0 + jnp.tanh(k * (x + 0.044715 * (x * x * x))))


def _dot(a, b):
    return jnp.dot(a, b, preferred_element_type=jnp.float32)


def _dot_nt(a, b):
    return lax.dot_general(a, b, _NT, preferred_element_type=jnp.float32)


def _head_diag_mask():
    r = lax.broadcasted_iota(jnp.int32, (_NBLK * _H, _ROWS), 0)
    c = lax.broadcasted_iota(jnp.int32, (_NBLK * _H, _ROWS), 1)
    return (r % _H) == (c % _H)


def _per_head_in(a, e_ref, w_ref):
    a_stack = jnp.concatenate(
        [a[:, b * _BLK:(b + 1) * _BLK] for b in range(_NBLK)], axis=0)
    y = _dot(a_stack, e_ref[...])
    lhs = jnp.where(_head_diag_mask(), y, 0.0).astype(jnp.bfloat16)
    out = jnp.zeros((_H, _D), jnp.float32)
    for b in range(_NBLK):
        out += _dot(lhs[b * _H:(b + 1) * _H], w_ref[b * _ROWS:(b + 1) * _ROWS, :])
    return out


def _per_head_out(q, scale, e_ref, w_ref):
    full = jnp.concatenate(
        [_dot_nt(q, w_ref[b * _ROWS:(b + 1) * _ROWS, :]) for b in range(_NBLK)],
        axis=0)
    diag = jnp.where(_head_diag_mask(), full * scale, 0.0).astype(jnp.bfloat16)
    stack = _dot_nt(diag, e_ref[...]).astype(jnp.bfloat16)
    return jnp.concatenate(
        [stack[b * _H:(b + 1) * _H] for b in range(_NBLK)], axis=1)


def _kernel(x_hbm, ckv_hbm, wq_hbm, wuk_hbm, wuv_hbm, wo_hbm, wg_hbm, wu_hbm,
            wd_hbm, c_hbm, wmod_hbm, o_ref,
            x_v, c_v, wmod_a, wmod_b, wq_v, wuk_v, ckv_v, wuv_v, wo_v, wg_v,
            wu_v, wd_v, e_v, sems, kv_sems, wd_sems):

    def kv_copy(i):
        rows = pl.ds(pl.multiple_of(i * _T, _T), _T)
        return pltpu.make_async_copy(ckv_hbm.at[rows, :], ckv_v.at[rows, :],
                                     kv_sems.at[i])

    def wd_copy(i):
        rows = pl.ds(_WD_SPLITS[i], _WD_SPLITS[i + 1] - _WD_SPLITS[i])
        return pltpu.make_async_copy(wd_hbm.at[rows, :], wd_v.at[rows, :],
                                     wd_sems.at[i])

    cp_moda = pltpu.make_async_copy(wmod_hbm.at[:, pl.ds(0, 2 * _M)], wmod_a, sems.at[0])
    cp_c = pltpu.make_async_copy(c_hbm, c_v, sems.at[1])
    cp_x = pltpu.make_async_copy(x_hbm, x_v, sems.at[2])
    cp_wq = pltpu.make_async_copy(wq_hbm, wq_v, sems.at[3])
    cp_wuk = pltpu.make_async_copy(wuk_hbm, wuk_v, sems.at[4])
    cp_wuv = pltpu.make_async_copy(wuv_hbm, wuv_v, sems.at[5])
    cp_wo = pltpu.make_async_copy(wo_hbm, wo_v, sems.at[6])
    cp_modb = pltpu.make_async_copy(wmod_hbm.at[:, pl.ds(2 * _M, 4 * _M)], wmod_b, sems.at[7])
    cp_wg = pltpu.make_async_copy(wg_hbm, wg_v, sems.at[8])
    cp_wu = pltpu.make_async_copy(wu_hbm, wu_v, sems.at[9])

    cp_moda.start()
    cp_c.start()
    cp_x.start()
    cp_wq.start()
    cp_wuk.start()
    for i in range(_NCHUNK):
        kv_copy(i).start()
    cp_wuv.start()
    cp_wo.start()
    cp_modb.start()
    cp_wg.start()
    cp_wu.start()
    for i in range(len(_WD_SPLITS) - 1):
        wd_copy(i).start()

    er = lax.broadcasted_iota(jnp.int32, (_BLK, _ROWS), 0)
    ec = lax.broadcasted_iota(jnp.int32, (_BLK, _ROWS), 1)
    e_v[...] = jnp.where(er == ec // _H, 1.0, 0.0).astype(jnp.bfloat16)

    cp_c.wait()
    cf = c_v[...].astype(jnp.float32)
    sc = (cf * jax.nn.sigmoid(cf)).astype(jnp.bfloat16)
    cp_moda.wait()
    mod_a = _dot(sc, wmod_a[...])
    cp_x.wait()
    x = x_v[...].astype(jnp.float32)
    h = _layernorm(x) * (1.0 + mod_a[:, _M:]) + mod_a[:, :_M]
    h = jnp.broadcast_to(h, (_H, _M)).astype(jnp.bfloat16)

    cp_wq.wait()
    q = _per_head_in(h, e_v, wq_v).astype(jnp.bfloat16)
    cp_wuk.wait()
    q_abs = _per_head_out(q, _D ** -0.5, e_v, wuk_v)

    def kv_step(i, carry):
        m, l, acc = carry
        kv_copy(i).wait()
        ckv = ckv_v[pl.ds(pl.multiple_of(i * _T, _T), _T), :]
        s = _dot_nt(q_abs, ckv)
        m_new = jnp.maximum(m, jnp.max(s, axis=1, keepdims=True))
        alpha = jnp.exp(m - m_new)
        p = jnp.exp(s - m_new)
        l = alpha * l + jnp.sum(p, axis=1, keepdims=True)
        acc = alpha * acc + _dot(p.astype(jnp.bfloat16), ckv)
        return m_new, l, acc

    _, l, acc = lax.fori_loop(
        0, _NCHUNK, kv_step,
        (jnp.full((_H, 1), -jnp.inf, jnp.float32),
         jnp.zeros((_H, 1), jnp.float32),
         jnp.zeros((_H, _M), jnp.float32)))
    ctx_c = (acc / l).astype(jnp.bfloat16)

    cp_wuv.wait()
    ctx = _per_head_in(ctx_c, e_v, wuv_v)
    hr = lax.broadcasted_iota(jnp.int32, (_H, _H * _D), 0)
    hc = lax.broadcasted_iota(jnp.int32, (_H, _H * _D), 1)
    lhs = jnp.where(hr == hc // _D, jnp.concatenate([ctx] * _H, axis=1), 0.0)
    cp_wo.wait()
    attn = jnp.sum(_dot(lhs.astype(jnp.bfloat16), wo_v[...]), axis=0, keepdims=True)

    cp_modb.wait()
    mod_b = _dot(sc, wmod_b[...])
    x1 = x + mod_b[:, :_M] * attn
    h2 = _layernorm(x1) * (1.0 + mod_b[:, 2 * _M:3 * _M]) + mod_b[:, _M:2 * _M]
    h2 = h2.astype(jnp.bfloat16)

    cp_wg.wait()
    g = _dot(h2, wg_v[...])
    cp_wu.wait()
    u = _dot(h2, wu_v[...])
    act = (_gelu_tanh(g) * u).astype(jnp.bfloat16)
    y = jnp.zeros((1, _M), jnp.float32)
    for i in range(len(_WD_SPLITS) - 1):
        lo, hi = _WD_SPLITS[i], _WD_SPLITS[i + 1]
        wd_copy(i).wait()
        y += _dot(act[:, lo:hi], wd_v[lo:hi, :])
    o_ref[...] = (x1 + mod_b[:, 3 * _M:] * y).astype(o_ref.dtype)


@jax.jit
def pallas_adaLN_cond__compressed_kv_cla__glu_gated_geglu__decode_kernel(
A_x: jax.Array,
    A_c_kv: jax.Array,
    A_w_q: jax.Array,
    A_w_uk: jax.Array,
    A_w_uv: jax.Array,
    A_w_o: jax.Array,
    B_x: jax.Array,
    B_w_gate: jax.Array,
    B_w_up: jax.Array,
    B_w_down: jax.Array,
    c: jax.Array,
    w_mod: jax.Array,
):
    del B_x
    bf16 = jnp.bfloat16
    any_spec = pl.BlockSpec(memory_space=pl.ANY)
    out = pl.pallas_call(
        _kernel,
        in_specs=[any_spec] * 11,
        out_specs=pl.BlockSpec(memory_space=pltpu.VMEM),
        out_shape=jax.ShapeDtypeStruct((1, _M), A_x.dtype),
        scratch_shapes=[
            pltpu.VMEM((1, _M), bf16),
            pltpu.VMEM((1, _M), bf16),
            pltpu.VMEM((_M, 2 * _M), bf16),
            pltpu.VMEM((_M, 4 * _M), bf16),
            pltpu.VMEM((_M * _H, _D), bf16),
            pltpu.VMEM((_M * _H, _D), bf16),
            pltpu.VMEM((_SK, _M), bf16),
            pltpu.VMEM((_M * _H, _D), bf16),
            pltpu.VMEM((_H * _D, _M), bf16),
            pltpu.VMEM((_M, _F), bf16),
            pltpu.VMEM((_M, _F), bf16),
            pltpu.VMEM((_F, _M), bf16),
            pltpu.VMEM((_BLK, _ROWS), bf16),
            pltpu.SemaphoreType.DMA((10,)),
            pltpu.SemaphoreType.DMA((_NCHUNK,)),
            pltpu.SemaphoreType.DMA((len(_WD_SPLITS) - 1,)),
        ],
        compiler_params=pltpu.CompilerParams(vmem_limit_bytes=100 * 1024 * 1024),
    )(
        A_x.reshape(1, _M),
        A_c_kv.reshape(_SK, _M),
        A_w_q.reshape(_M * _H, _D),
        A_w_uk.reshape(_M * _H, _D),
        A_w_uv.reshape(_M * _H, _D),
        A_w_o.reshape(_H * _D, _M),
        B_w_gate,
        B_w_up,
        B_w_down,
        c,
        w_mod,
    )
    return out.reshape(1, 1, _M)
```

```python
import functools

import jax
import jax.numpy as jnp
from jax import lax
import jax.experimental.pallas as pl
import jax.experimental.pallas.tpu as pltpu

_H = 32
_D = 128
_M = 512
_F = 1792
_SK = 32768
_T = 4096
_NCHUNK = _SK // _T
_BLK = 128
_ROWS = _BLK * _H
_NBLK = _M // _BLK
_WD_SPLITS = (0, 1024, 1536, 1792)
_EPS = 1e-5
_NT = (((1,), (1,)), ((), ()))


def _layernorm(x):
    mean = jnp.mean(x, axis=-1, keepdims=True)
    xc = x - mean
    var = jnp.mean(xc * xc, axis=-1, keepdims=True)
    return xc / jnp.sqrt(var + _EPS)


def _gelu_tanh(x):
    k = 0.7978845608028654
    return 0.5 * x * (1.0 + jnp.tanh(k * (x + 0.044715 * (x * x * x))))


def _dot(a, b):
    return jnp.dot(a, b, preferred_element_type=jnp.float32)


def _dot_nt(a, b):
    return lax.dot_general(a, b, _NT, preferred_element_type=jnp.float32)


def _head_diag_mask():
    r = lax.broadcasted_iota(jnp.int32, (_NBLK * _H, _ROWS), 0)
    c = lax.broadcasted_iota(jnp.int32, (_NBLK * _H, _ROWS), 1)
    return (r % _H) == (c % _H)


def _per_head_in(a, e_ref, w_ref):
    a_stack = jnp.concatenate(
        [a[:, b * _BLK:(b + 1) * _BLK] for b in range(_NBLK)], axis=0)
    y = _dot(a_stack, e_ref[...])
    lhs = jnp.where(_head_diag_mask(), y, 0.0).astype(jnp.bfloat16)
    out = jnp.zeros((_H, _D), jnp.float32)
    for b in range(_NBLK):
        out += _dot(lhs[b * _H:(b + 1) * _H], w_ref[b * _ROWS:(b + 1) * _ROWS, :])
    return out


def _per_head_out(q, scale, e_ref, w_ref):
    full = jnp.concatenate(
        [_dot_nt(q, w_ref[b * _ROWS:(b + 1) * _ROWS, :]) for b in range(_NBLK)],
        axis=0)
    diag = jnp.where(_head_diag_mask(), full * scale, 0.0).astype(jnp.bfloat16)
    stack = _dot_nt(diag, e_ref[...]).astype(jnp.bfloat16)
    return jnp.concatenate(
        [stack[b * _H:(b + 1) * _H] for b in range(_NBLK)], axis=1)


def _kernel(x_hbm, ckv_hbm, wq_hbm, wuk_hbm, wuv_hbm, wo_hbm, wg_hbm, wu_hbm,
            wd_hbm, c_hbm, wmod_hbm, o_ref,
            x_v, c_v, wmod_a, wmod_b, wq_v, wuk_v, ckv_v, wuv_v, wo_v, wg_v,
            wu_v, wd_v, e_v, sems):

    def kv_copy(i):
        rows = pl.ds(pl.multiple_of(i * _T, _T), _T)
        return pltpu.make_async_copy(ckv_hbm.at[rows, :], ckv_v.at[rows, :],
                                     sems.at[10 + i])

    def wd_copy(i):
        rows = pl.ds(_WD_SPLITS[i], _WD_SPLITS[i + 1] - _WD_SPLITS[i])
        return pltpu.make_async_copy(wd_hbm.at[rows, :], wd_v.at[rows, :],
                                     sems.at[10 + _NCHUNK + i])

    cp_moda = pltpu.make_async_copy(wmod_hbm.at[:, pl.ds(0, 2 * _M)], wmod_a, sems.at[0])
    cp_c = pltpu.make_async_copy(c_hbm, c_v, sems.at[1])
    cp_x = pltpu.make_async_copy(x_hbm, x_v, sems.at[2])
    cp_wq = pltpu.make_async_copy(wq_hbm, wq_v, sems.at[3])
    cp_wuk = pltpu.make_async_copy(wuk_hbm, wuk_v, sems.at[4])
    cp_wuv = pltpu.make_async_copy(wuv_hbm, wuv_v, sems.at[5])
    cp_wo = pltpu.make_async_copy(wo_hbm, wo_v, sems.at[6])
    cp_modb = pltpu.make_async_copy(wmod_hbm.at[:, pl.ds(2 * _M, 4 * _M)], wmod_b, sems.at[7])
    cp_wg = pltpu.make_async_copy(wg_hbm, wg_v, sems.at[8])
    cp_wu = pltpu.make_async_copy(wu_hbm, wu_v, sems.at[9])

    cp_moda.start()
    cp_c.start()
    cp_x.start()
    cp_wq.start()
    cp_wuk.start()
    for i in range(_NCHUNK):
        kv_copy(i).start()
    cp_wuv.start()
    cp_wo.start()
    cp_modb.start()
    cp_wg.start()
    cp_wu.start()
    for i in range(len(_WD_SPLITS) - 1):
        wd_copy(i).start()

    er = lax.broadcasted_iota(jnp.int32, (_BLK, _ROWS), 0)
    ec = lax.broadcasted_iota(jnp.int32, (_BLK, _ROWS), 1)
    e_v[...] = jnp.where(er == ec // _H, 1.0, 0.0).astype(jnp.bfloat16)

    cp_c.wait()
    cf = c_v[...].astype(jnp.float32)
    sc = (cf * jax.nn.sigmoid(cf)).astype(jnp.bfloat16)
    cp_moda.wait()
    mod_a = _dot(sc, wmod_a[...])
    cp_x.wait()
    x = x_v[...].astype(jnp.float32)
    h = _layernorm(x) * (1.0 + mod_a[:, _M:]) + mod_a[:, :_M]
    h = jnp.broadcast_to(h, (_H, _M)).astype(jnp.bfloat16)

    cp_wq.wait()
    q = _per_head_in(h, e_v, wq_v).astype(jnp.bfloat16)
    cp_wuk.wait()
    q_abs = _per_head_out(q, _D ** -0.5, e_v, wuk_v)

    def kv_step(i, carry):
        m, l, acc = carry
        kv_copy(i).wait()
        ckv = ckv_v[pl.ds(pl.multiple_of(i * _T, _T), _T), :]
        s = _dot_nt(q_abs, ckv)
        m_new = jnp.maximum(m, jnp.max(s, axis=1, keepdims=True))
        alpha = jnp.exp(m - m_new)
        p = jnp.exp(s - m_new)
        l = alpha * l + jnp.sum(p, axis=1, keepdims=True)
        acc = alpha * acc + _dot(p.astype(jnp.bfloat16), ckv)
        return m_new, l, acc

    _, l, acc = lax.fori_loop(
        0, _NCHUNK, kv_step,
        (jnp.full((_H, 1), -jnp.inf, jnp.float32),
         jnp.zeros((_H, 1), jnp.float32),
         jnp.zeros((_H, _M), jnp.float32)))
    ctx_c = (acc / l).astype(jnp.bfloat16)

    cp_wuv.wait()
    ctx = _per_head_in(ctx_c, e_v, wuv_v)
    hr = lax.broadcasted_iota(jnp.int32, (_H, _H * _D), 0)
    hc = lax.broadcasted_iota(jnp.int32, (_H, _H * _D), 1)
    lhs = jnp.where(hr == hc // _D, jnp.concatenate([ctx] * _H, axis=1), 0.0)
    cp_wo.wait()
    attn = jnp.sum(_dot(lhs.astype(jnp.bfloat16), wo_v[...]), axis=0, keepdims=True)

    cp_modb.wait()
    mod_b = _dot(sc, wmod_b[...])
    x1 = x + mod_b[:, :_M] * attn
    h2 = _layernorm(x1) * (1.0 + mod_b[:, 2 * _M:3 * _M]) + mod_b[:, _M:2 * _M]
    h2 = h2.astype(jnp.bfloat16)

    cp_wg.wait()
    g = _dot(h2, wg_v[...])
    cp_wu.wait()
    u = _dot(h2, wu_v[...])
    act = (_gelu_tanh(g) * u).astype(jnp.bfloat16)
    y = jnp.zeros((1, _M), jnp.float32)
    for i in range(len(_WD_SPLITS) - 1):
        lo, hi = _WD_SPLITS[i], _WD_SPLITS[i + 1]
        wd_copy(i).wait()
        y += _dot(act[:, lo:hi], wd_v[lo:hi, :])
    o_ref[...] = (x1 + mod_b[:, 3 * _M:] * y).astype(o_ref.dtype)


@jax.jit
def pallas_adaLN_cond__compressed_kv_cla__glu_gated_geglu__decode_kernel(
A_x: jax.Array,
    A_c_kv: jax.Array,
    A_w_q: jax.Array,
    A_w_uk: jax.Array,
    A_w_uv: jax.Array,
    A_w_o: jax.Array,
    B_x: jax.Array,
    B_w_gate: jax.Array,
    B_w_up: jax.Array,
    B_w_down: jax.Array,
    c: jax.Array,
    w_mod: jax.Array,
):
    del B_x
    bf16 = jnp.bfloat16
    any_spec = pl.BlockSpec(memory_space=pl.ANY)
    out = pl.pallas_call(
        _kernel,
        in_specs=[any_spec] * 11,
        out_specs=pl.BlockSpec(memory_space=pltpu.VMEM),
        out_shape=jax.ShapeDtypeStruct((1, _M), A_x.dtype),
        scratch_shapes=[
            pltpu.VMEM((1, _M), bf16),
            pltpu.VMEM((1, _M), bf16),
            pltpu.VMEM((_M, 2 * _M), bf16),
            pltpu.VMEM((_M, 4 * _M), bf16),
            pltpu.VMEM((_M * _H, _D), bf16),
            pltpu.VMEM((_M * _H, _D), bf16),
            pltpu.VMEM((_SK, _M), bf16),
            pltpu.VMEM((_M * _H, _D), bf16),
            pltpu.VMEM((_H * _D, _M), bf16),
            pltpu.VMEM((_M, _F), bf16),
            pltpu.VMEM((_M, _F), bf16),
            pltpu.VMEM((_F, _M), bf16),
            pltpu.VMEM((_BLK, _ROWS), bf16),
            pltpu.SemaphoreType.DMA((10 + _NCHUNK + len(_WD_SPLITS) - 1,)),
        ],
        compiler_params=pltpu.CompilerParams(vmem_limit_bytes=100 * 1024 * 1024),
    )(
        A_x.reshape(1, _M),
        A_c_kv.reshape(_SK, _M),
        A_w_q.reshape(_M * _H, _D),
        A_w_uk.reshape(_M * _H, _D),
        A_w_uv.reshape(_M * _H, _D),
        A_w_o.reshape(_H * _D, _M),
        B_w_gate,
        B_w_up,
        B_w_down,
        c,
        w_mod,
    )
    return out.reshape(1, 1, _M)
```

```python
import contextlib

import jax
import jax.numpy as jnp
from jax import lax
import jax.experimental.pallas as pl
import jax.experimental.pallas.tpu as pltpu

_H = 32
_D = 128
_M = 512
_F = 1792
_SK = 32768
_T = 4096
_NCHUNK = _SK // _T
_BLK = 128
_ROWS = _BLK * _H
_NBLK = _M // _BLK
_KV_SPLITS = (0, 3, 6, 8)
_NKV = len(_KV_SPLITS) - 1
_WD_SPLITS = (0, 1152, 1664, 1792)
_EPS = 1e-5
_NT = (((1,), (1,)), ((), ()))


_PROFILE = False


def _scope(name):
    return jax.named_scope(name) if _PROFILE else contextlib.nullcontext()


def _layernorm(x):
    mean = jnp.mean(x, axis=-1, keepdims=True)
    xc = x - mean
    var = jnp.mean(xc * xc, axis=-1, keepdims=True)
    return xc / jnp.sqrt(var + _EPS)


def _gelu_tanh(x):
    k = 0.7978845608028654
    return 0.5 * x * (1.0 + jnp.tanh(k * (x + 0.044715 * (x * x * x))))


def _dot(a, b):
    return jnp.dot(a, b, preferred_element_type=jnp.float32)


def _dot_nt(a, b):
    return lax.dot_general(a, b, _NT, preferred_element_type=jnp.float32)


def _head_diag_mask():
    r = lax.broadcasted_iota(jnp.int32, (_NBLK * _H, _ROWS), 0)
    c = lax.broadcasted_iota(jnp.int32, (_NBLK * _H, _ROWS), 1)
    return (r % _H) == (c % _H)


def _per_head_in(a, e_ref, w_ref):
    a_stack = jnp.concatenate(
        [a[:, b * _BLK:(b + 1) * _BLK] for b in range(_NBLK)], axis=0)
    y = _dot(a_stack, e_ref[...])
    lhs = jnp.where(_head_diag_mask(), y, 0.0).astype(jnp.bfloat16)
    out = jnp.zeros((_H, _D), jnp.float32)
    for b in range(_NBLK):
        out += _dot(lhs[b * _H:(b + 1) * _H], w_ref[b * _ROWS:(b + 1) * _ROWS, :])
    return out


def _per_head_out(q, scale, e_ref, w_ref):
    full = jnp.concatenate(
        [_dot_nt(q, w_ref[b * _ROWS:(b + 1) * _ROWS, :]) for b in range(_NBLK)],
        axis=0)
    diag = jnp.where(_head_diag_mask(), full * scale, 0.0).astype(jnp.bfloat16)
    stack = _dot_nt(diag, e_ref[...]).astype(jnp.bfloat16)
    return jnp.concatenate(
        [stack[b * _H:(b + 1) * _H] for b in range(_NBLK)], axis=1)


def _kernel(x_hbm, ckv_hbm, wq_hbm, wuk_hbm, wuv_hbm, wo_hbm, wg_hbm, wu_hbm,
            wd_hbm, c_hbm, wmod_hbm, o_ref,
            x_v, c_v, wmod_v, wq_v, wuk_v, ckv_v, wuv_v, wo_v, wg_v,
            wu_v, e_v, y_v, sems, *wd_v):

    def kv_copy(i):
        rows = pl.ds(_KV_SPLITS[i] * _T, (_KV_SPLITS[i + 1] - _KV_SPLITS[i]) * _T)
        return pltpu.make_async_copy(ckv_hbm.at[rows, :], ckv_v.at[rows, :],
                                     sems.at[9 + i])

    def wd_copy(i):
        rows = pl.ds(_WD_SPLITS[i], _WD_SPLITS[i + 1] - _WD_SPLITS[i])
        return pltpu.make_async_copy(wd_hbm.at[rows, :], wd_v[i],
                                     sems.at[9 + _NKV + i])

    cp_mod = pltpu.make_async_copy(wmod_hbm, wmod_v, sems.at[0])
    cp_c = pltpu.make_async_copy(c_hbm, c_v, sems.at[1])
    cp_x = pltpu.make_async_copy(x_hbm, x_v, sems.at[2])
    cp_wq = pltpu.make_async_copy(wq_hbm, wq_v, sems.at[3])
    cp_wuk = pltpu.make_async_copy(wuk_hbm, wuk_v, sems.at[4])
    cp_wuv = pltpu.make_async_copy(wuv_hbm, wuv_v, sems.at[5])
    cp_wo = pltpu.make_async_copy(wo_hbm, wo_v, sems.at[6])
    cp_wg = pltpu.make_async_copy(wg_hbm, wg_v, sems.at[7])
    cp_wu = pltpu.make_async_copy(wu_hbm, wu_v, sems.at[8])

    cp_mod.start()
    cp_c.start()
    cp_x.start()
    cp_wq.start()
    cp_wuk.start()
    for i in range(_NKV):
        kv_copy(i).start()
    cp_wuv.start()
    cp_wo.start()
    cp_wg.start()
    cp_wu.start()
    for i in range(len(_WD_SPLITS) - 1):
        wd_copy(i).start()

    with _scope("mk_e"):
        er = lax.broadcasted_iota(jnp.int32, (_BLK, _ROWS), 0)
        ec = lax.broadcasted_iota(jnp.int32, (_BLK, _ROWS), 1)
        e_v[...] = jnp.where(er == ec // _H, 1.0, 0.0).astype(jnp.bfloat16)

    with _scope("w_mod"):
        cp_c.wait()
        cp_x.wait()
        cp_mod.wait()
    with _scope("c_mod"):
        cf = c_v[...].astype(jnp.float32)
        sc = (cf * jax.nn.sigmoid(cf)).astype(jnp.bfloat16)
        mod_a = _dot(sc, wmod_v[:, :2 * _M])
        x = x_v[...].astype(jnp.float32)
        h = _layernorm(x) * (1.0 + mod_a[:, _M:]) + mod_a[:, :_M]
        h = jnp.broadcast_to(h, (_H, _M)).astype(jnp.bfloat16)
        mod_b = _dot(sc, wmod_v[:, 2 * _M:])

    with _scope("w_q"):
        cp_wq.wait()
    with _scope("c_q"):
        q = _per_head_in(h, e_v, wq_v).astype(jnp.bfloat16)
    with _scope("w_uk"):
        cp_wuk.wait()
    with _scope("c_uk"):
        q_abs = _per_head_out(q, _D ** -0.5, e_v, wuk_v)

    def kv_step(i, carry):
        m, l, acc = carry
        with _scope("w_kv"):
            for j in range(_NKV):
                pl.when(i == _KV_SPLITS[j])(kv_copy(j).wait)
        with _scope("c_kv"):
            ckv = ckv_v[pl.ds(pl.multiple_of(i * _T, _T), _T), :]
            s = _dot_nt(q_abs, ckv)
            m_new = jnp.maximum(m, jnp.max(s, axis=1, keepdims=True))
            alpha = jnp.exp(m - m_new)
            p = jnp.exp(s - m_new)
            l = alpha * l + jnp.sum(p, axis=1, keepdims=True)
            acc = alpha * acc + _dot(p.astype(jnp.bfloat16), ckv)
        return m_new, l, acc

    _, l, acc = lax.fori_loop(
        0, _NCHUNK, kv_step,
        (jnp.full((_H, 1), -jnp.inf, jnp.float32),
         jnp.zeros((_H, 1), jnp.float32),
         jnp.zeros((_H, _M), jnp.float32)))
    ctx_c = (acc / l).astype(jnp.bfloat16)

    with _scope("w_uv"):
        cp_wuv.wait()
    with _scope("c_uv"):
        ctx = _per_head_in(ctx_c, e_v, wuv_v)
        hr = lax.broadcasted_iota(jnp.int32, (_H, _H * _D), 0)
        hc = lax.broadcasted_iota(jnp.int32, (_H, _H * _D), 1)
        lhs = jnp.where(hr == hc // _D, jnp.concatenate([ctx] * _H, axis=1), 0.0)
        lhs = lhs.astype(jnp.bfloat16)
    with _scope("w_o"):
        cp_wo.wait()
    with _scope("c_o"):
        attn = jnp.sum(_dot(lhs, wo_v[...]), axis=0, keepdims=True)
        x1 = x + mod_b[:, :_M] * attn
        h2 = _layernorm(x1) * (1.0 + mod_b[:, 2 * _M:3 * _M]) + mod_b[:, _M:2 * _M]
        h2 = h2.astype(jnp.bfloat16)

    with _scope("w_g"):
        cp_wg.wait()
    with _scope("c_g"):
        g = _gelu_tanh(_dot(h2, wg_v[...]))
    with _scope("w_u"):
        cp_wu.wait()
    with _scope("c_u"):
        act = (g * _dot(h2, wu_v[...])).astype(jnp.bfloat16)
    n_wd = len(_WD_SPLITS) - 1
    for i in range(n_wd):
        lo, hi = _WD_SPLITS[i], _WD_SPLITS[i + 1]
        with _scope("w_d%d" % i):
            wd_copy(i).wait()
        with _scope("c_d%d" % i):
            part = _dot(act[:, lo:hi], wd_v[i][...])
            if i == 0:
                y_v[...] = part
            elif i < n_wd - 1:
                y_v[...] += part
    o_ref[...] = (x1 + mod_b[:, 3 * _M:] * (y_v[...] + part)).astype(o_ref.dtype)


@jax.jit
def pallas_adaLN_cond__compressed_kv_cla__glu_gated_geglu__decode_kernel(
A_x: jax.Array,
    A_c_kv: jax.Array,
    A_w_q: jax.Array,
    A_w_uk: jax.Array,
    A_w_uv: jax.Array,
    A_w_o: jax.Array,
    B_x: jax.Array,
    B_w_gate: jax.Array,
    B_w_up: jax.Array,
    B_w_down: jax.Array,
    c: jax.Array,
    w_mod: jax.Array,
):
    del B_x
    bf16 = jnp.bfloat16
    any_spec = pl.BlockSpec(memory_space=pl.ANY)
    out = pl.pallas_call(
        _kernel,
        in_specs=[any_spec] * 11,
        out_specs=pl.BlockSpec(memory_space=pltpu.VMEM),
        out_shape=jax.ShapeDtypeStruct((1, _M), A_x.dtype),
        scratch_shapes=[
            pltpu.VMEM((1, _M), bf16),
            pltpu.VMEM((1, _M), bf16),
            pltpu.VMEM((_M, 6 * _M), bf16),
            pltpu.VMEM((_M * _H, _D), bf16),
            pltpu.VMEM((_M * _H, _D), bf16),
            pltpu.VMEM((_SK, _M), bf16),
            pltpu.VMEM((_M * _H, _D), bf16),
            pltpu.VMEM((_H * _D, _M), bf16),
            pltpu.VMEM((_M, _F), bf16),
            pltpu.VMEM((_M, _F), bf16),
            pltpu.VMEM((_BLK, _ROWS), bf16),
            pltpu.VMEM((1, _M), jnp.float32),
            pltpu.SemaphoreType.DMA((9 + _NKV + len(_WD_SPLITS) - 1,)),
        ] + [pltpu.VMEM((hi - lo, _M), bf16)
             for lo, hi in zip(_WD_SPLITS[:-1], _WD_SPLITS[1:])],
        compiler_params=pltpu.CompilerParams(vmem_limit_bytes=100 * 1024 * 1024),
    )(
        A_x.reshape(1, _M),
        A_c_kv.reshape(_SK, _M),
        A_w_q.reshape(_M * _H, _D),
        A_w_uk.reshape(_M * _H, _D),
        A_w_uv.reshape(_M * _H, _D),
        A_w_o.reshape(_H * _D, _M),
        B_w_gate,
        B_w_up,
        B_w_down,
        c,
        w_mod,
    )
    return out.reshape(1, 1, _M)
```

```python
import contextlib

import jax
import jax.numpy as jnp
from jax import lax
import jax.experimental.pallas as pl
import jax.experimental.pallas.tpu as pltpu

_H = 32
_D = 128
_M = 512
_F = 1792
_SK = 32768
_T = 4096
_NCHUNK = _SK // _T
_BLK = 128
_ROWS = _BLK * _H
_NBLK = _M // _BLK
_KV_SPLITS = (0, 3, 6, 8)
_NKV = len(_KV_SPLITS) - 1
_WD_SPLITS = (0, 1280, 1664, 1792)
_EPS = 1e-5
_NT = (((1,), (1,)), ((), ()))


_PROFILE = False


def _scope(name):
    return jax.named_scope(name) if _PROFILE else contextlib.nullcontext()


def _layernorm(x):
    mean = jnp.mean(x, axis=-1, keepdims=True)
    xc = x - mean
    var = jnp.mean(xc * xc, axis=-1, keepdims=True)
    return xc / jnp.sqrt(var + _EPS)


def _gelu_tanh(x):
    k = 0.7978845608028654
    return 0.5 * x * (1.0 + jnp.tanh(k * (x + 0.044715 * (x * x * x))))


def _dot(a, b):
    return jnp.dot(a, b, preferred_element_type=jnp.float32)


def _dot_nt(a, b):
    return lax.dot_general(a, b, _NT, preferred_element_type=jnp.float32)


def _head_diag_mask():
    r = lax.broadcasted_iota(jnp.int32, (_NBLK * _H, _ROWS), 0)
    c = lax.broadcasted_iota(jnp.int32, (_NBLK * _H, _ROWS), 1)
    return (r % _H) == (c % _H)


def _per_head_in(a, e_ref, w_ref):
    a_stack = jnp.concatenate(
        [a[:, b * _BLK:(b + 1) * _BLK] for b in range(_NBLK)], axis=0)
    y = _dot(a_stack, e_ref[...])
    lhs = jnp.where(_head_diag_mask(), y, 0.0).astype(jnp.bfloat16)
    out = jnp.zeros((_H, _D), jnp.float32)
    for b in range(_NBLK):
        out += _dot(lhs[b * _H:(b + 1) * _H], w_ref[b * _ROWS:(b + 1) * _ROWS, :])
    return out


def _per_head_out(q, scale, e_ref, w_ref):
    full = jnp.concatenate(
        [_dot_nt(q, w_ref[b * _ROWS:(b + 1) * _ROWS, :]) for b in range(_NBLK)],
        axis=0)
    diag = jnp.where(_head_diag_mask(), full * scale, 0.0).astype(jnp.bfloat16)
    stack = _dot_nt(diag, e_ref[...]).astype(jnp.bfloat16)
    return jnp.concatenate(
        [stack[b * _H:(b + 1) * _H] for b in range(_NBLK)], axis=1)


def _kernel(x_hbm, ckv_hbm, wq_hbm, wuk_hbm, wuv_hbm, wo_hbm, wg_hbm, wu_hbm,
            wd_hbm, c_hbm, wmod_hbm, o_ref,
            x_v, c_v, wmod_v, wq_v, wuk_v, ckv_v, wuv_v, wo_v, wg_v,
            wu_v, e_v, y_v, acol_v, sems, *wd_v):

    def kv_copy(i):
        rows = pl.ds(_KV_SPLITS[i] * _T, (_KV_SPLITS[i + 1] - _KV_SPLITS[i]) * _T)
        return pltpu.make_async_copy(ckv_hbm.at[rows, :], ckv_v.at[rows, :],
                                     sems.at[9 + i])

    def wd_copy(i):
        rows = pl.ds(_WD_SPLITS[i], _WD_SPLITS[i + 1] - _WD_SPLITS[i])
        return pltpu.make_async_copy(wd_hbm.at[rows, :], wd_v[i],
                                     sems.at[9 + _NKV + i])

    cp_mod = pltpu.make_async_copy(wmod_hbm, wmod_v, sems.at[0])
    cp_c = pltpu.make_async_copy(c_hbm, c_v, sems.at[1])
    cp_x = pltpu.make_async_copy(x_hbm, x_v, sems.at[2])
    cp_wq = pltpu.make_async_copy(wq_hbm, wq_v, sems.at[3])
    cp_wuk = pltpu.make_async_copy(wuk_hbm, wuk_v, sems.at[4])
    cp_wuv = pltpu.make_async_copy(wuv_hbm, wuv_v, sems.at[5])
    cp_wo = pltpu.make_async_copy(wo_hbm, wo_v, sems.at[6])
    cp_wg = pltpu.make_async_copy(wg_hbm, wg_v, sems.at[7])
    cp_wu = pltpu.make_async_copy(wu_hbm, wu_v, sems.at[8])

    cp_mod.start()
    cp_c.start()
    cp_x.start()
    cp_wq.start()
    cp_wuk.start()
    for i in range(_NKV):
        kv_copy(i).start()
    cp_wuv.start()
    cp_wo.start()
    cp_wg.start()
    cp_wu.start()
    for i in range(len(_WD_SPLITS) - 1):
        wd_copy(i).start()

    with _scope("mk_e"):
        er = lax.broadcasted_iota(jnp.int32, (_BLK, _ROWS), 0)
        ec = lax.broadcasted_iota(jnp.int32, (_BLK, _ROWS), 1)
        e_v[...] = jnp.where(er == ec // _H, 1.0, 0.0).astype(jnp.bfloat16)

    with _scope("w_mod"):
        cp_c.wait()
        cp_x.wait()
        cp_mod.wait()
    with _scope("c_mod"):
        cf = c_v[...].astype(jnp.float32)
        sc = (cf * jax.nn.sigmoid(cf)).astype(jnp.bfloat16)
        mod_a = _dot(sc, wmod_v[:, :2 * _M])
        x = x_v[...].astype(jnp.float32)
        h = _layernorm(x) * (1.0 + mod_a[:, _M:]) + mod_a[:, :_M]
        h = jnp.broadcast_to(h, (_H, _M)).astype(jnp.bfloat16)
        mod_b = _dot(sc, wmod_v[:, 2 * _M:])

    with _scope("w_q"):
        cp_wq.wait()
    with _scope("c_q"):
        q = _per_head_in(h, e_v, wq_v).astype(jnp.bfloat16)
    with _scope("w_uk"):
        cp_wuk.wait()
    with _scope("c_uk"):
        q_abs = _per_head_out(q, _D ** -0.5, e_v, wuk_v)

    def kv_step(i, carry):
        m, l, acc = carry
        with _scope("w_kv"):
            for j in range(_NKV):
                pl.when(i == _KV_SPLITS[j])(kv_copy(j).wait)
        with _scope("c_kv"):
            ckv = ckv_v[pl.ds(pl.multiple_of(i * _T, _T), _T), :]
            s = _dot_nt(q_abs, ckv)
            m_new = jnp.maximum(m, jnp.max(s, axis=1, keepdims=True))
            alpha = jnp.exp(m - m_new)
            p = jnp.exp(s - m_new)
            l = alpha * l + jnp.sum(p, axis=1, keepdims=True)
            acc = alpha * acc + _dot(p.astype(jnp.bfloat16), ckv)
        return m_new, l, acc

    _, l, acc = lax.fori_loop(
        0, _NCHUNK, kv_step,
        (jnp.full((_H, 1), -jnp.inf, jnp.float32),
         jnp.zeros((_H, 1), jnp.float32),
         jnp.zeros((_H, _M), jnp.float32)))
    ctx_c = (acc / l).astype(jnp.bfloat16)

    with _scope("w_uv"):
        cp_wuv.wait()
    with _scope("c_uv"):
        ctx = _per_head_in(ctx_c, e_v, wuv_v)
        hr = lax.broadcasted_iota(jnp.int32, (_H, _H * _D), 0)
        hc = lax.broadcasted_iota(jnp.int32, (_H, _H * _D), 1)
        lhs = jnp.where(hr == hc // _D, jnp.concatenate([ctx] * _H, axis=1), 0.0)
        lhs = lhs.astype(jnp.bfloat16)
    with _scope("w_o"):
        cp_wo.wait()
    with _scope("c_o"):
        attn = jnp.sum(_dot(lhs, wo_v[...]), axis=0, keepdims=True)
        x1 = x + mod_b[:, :_M] * attn
        h2 = _layernorm(x1) * (1.0 + mod_b[:, 2 * _M:3 * _M]) + mod_b[:, _M:2 * _M]
        h2 = h2.astype(jnp.bfloat16)

    with _scope("w_g"):
        cp_wg.wait()
    with _scope("c_g"):
        g = _gelu_tanh(_dot(h2, wg_v[...]))
    with _scope("w_u"):
        cp_wu.wait()
    with _scope("c_u"):
        act = (g * _dot(h2, wu_v[...])).astype(jnp.bfloat16)
    n_wd = len(_WD_SPLITS) - 1
    with _scope("c_acol"):
        lo = _WD_SPLITS[-2]
        a_last = act[:, lo:].astype(jnp.float32)
        acol_v[...] = jnp.broadcast_to(a_last, (128, _F - lo)).T
    for i in range(n_wd - 1):
        lo, hi = _WD_SPLITS[i], _WD_SPLITS[i + 1]
        with _scope("w_d%d" % i):
            wd_copy(i).wait()
        with _scope("c_d%d" % i):
            part = _dot(act[:, lo:hi], wd_v[i][...])
            if i == 0:
                y_v[...] = part
            elif i < n_wd - 2:
                y_v[...] += part
    gb = mod_b[:, 3 * _M:]
    y_v[...] = x1 + gb * (y_v[...] + part)
    with _scope("w_dl"):
        wd_copy(n_wd - 1).wait()
    with _scope("c_dl"):
        acol = acol_v[...]
        cols = []
        for n in range(_M // 128):
            w = wd_v[-1][:, n * 128:(n + 1) * 128].astype(jnp.float32)
            cols.append(jnp.sum(w * acol, axis=0, keepdims=True))
        y_last = jnp.concatenate(cols, axis=1)
        o_ref[...] = (y_v[...] + gb * y_last).astype(o_ref.dtype)


@jax.jit
def pallas_adaLN_cond__compressed_kv_cla__glu_gated_geglu__decode_kernel(
A_x: jax.Array,
    A_c_kv: jax.Array,
    A_w_q: jax.Array,
    A_w_uk: jax.Array,
    A_w_uv: jax.Array,
    A_w_o: jax.Array,
    B_x: jax.Array,
    B_w_gate: jax.Array,
    B_w_up: jax.Array,
    B_w_down: jax.Array,
    c: jax.Array,
    w_mod: jax.Array,
):
    del B_x
    bf16 = jnp.bfloat16
    any_spec = pl.BlockSpec(memory_space=pl.ANY)
    out = pl.pallas_call(
        _kernel,
        in_specs=[any_spec] * 11,
        out_specs=pl.BlockSpec(memory_space=pltpu.VMEM),
        out_shape=jax.ShapeDtypeStruct((1, _M), A_x.dtype),
        scratch_shapes=[
            pltpu.VMEM((1, _M), bf16),
            pltpu.VMEM((1, _M), bf16),
            pltpu.VMEM((_M, 6 * _M), bf16),
            pltpu.VMEM((_M * _H, _D), bf16),
            pltpu.VMEM((_M * _H, _D), bf16),
            pltpu.VMEM((_SK, _M), bf16),
            pltpu.VMEM((_M * _H, _D), bf16),
            pltpu.VMEM((_H * _D, _M), bf16),
            pltpu.VMEM((_M, _F), bf16),
            pltpu.VMEM((_M, _F), bf16),
            pltpu.VMEM((_BLK, _ROWS), bf16),
            pltpu.VMEM((1, _M), jnp.float32),
            pltpu.VMEM((_F - _WD_SPLITS[-2], 128), jnp.float32),
            pltpu.SemaphoreType.DMA((9 + _NKV + len(_WD_SPLITS) - 1,)),
        ] + [pltpu.VMEM((hi - lo, _M), bf16)
             for lo, hi in zip(_WD_SPLITS[:-1], _WD_SPLITS[1:])],
        compiler_params=pltpu.CompilerParams(vmem_limit_bytes=100 * 1024 * 1024),
    )(
        A_x.reshape(1, _M),
        A_c_kv.reshape(_SK, _M),
        A_w_q.reshape(_M * _H, _D),
        A_w_uk.reshape(_M * _H, _D),
        A_w_uv.reshape(_M * _H, _D),
        A_w_o.reshape(_H * _D, _M),
        B_w_gate,
        B_w_up,
        B_w_down,
        c,
        w_mod,
    )
    return out.reshape(1, 1, _M)
```

```python
import contextlib

import jax
import jax.numpy as jnp
from jax import lax
import jax.experimental.pallas as pl
import jax.experimental.pallas.tpu as pltpu

_H = 32
_D = 128
_M = 512
_F = 1792
_SK = 32768
_T = 4096
_NCHUNK = _SK // _T
_BLK = 128
_ROWS = _BLK * _H
_NBLK = _M // _BLK
_KV_SPLITS = (0, 5, 8)
_NKV = len(_KV_SPLITS) - 1
_WD_SPLITS = (0, 1280, 1664, 1792)
_EPS = 1e-5
_NT = (((1,), (1,)), ((), ()))


_PROFILE = False


def _scope(name):
    return jax.named_scope(name) if _PROFILE else contextlib.nullcontext()


def _layernorm(x):
    mean = jnp.mean(x, axis=-1, keepdims=True)
    xc = x - mean
    var = jnp.mean(xc * xc, axis=-1, keepdims=True)
    return xc / jnp.sqrt(var + _EPS)


def _gelu_tanh(x):
    k = 0.7978845608028654
    return 0.5 * x * (1.0 + jnp.tanh(k * (x + 0.044715 * (x * x * x))))


def _dot(a, b):
    return jnp.dot(a, b, preferred_element_type=jnp.float32)


def _dot_nt(a, b):
    return lax.dot_general(a, b, _NT, preferred_element_type=jnp.float32)


def _head_diag_mask():
    r = lax.broadcasted_iota(jnp.int32, (_NBLK * _H, _ROWS), 0)
    c = lax.broadcasted_iota(jnp.int32, (_NBLK * _H, _ROWS), 1)
    return (r % _H) == (c % _H)


def _per_head_in(a, e_ref, w_ref):
    a_stack = jnp.concatenate(
        [a[:, b * _BLK:(b + 1) * _BLK] for b in range(_NBLK)], axis=0)
    y = _dot(a_stack, e_ref[...])
    lhs = jnp.where(_head_diag_mask(), y, 0.0).astype(jnp.bfloat16)
    out = jnp.zeros((_H, _D), jnp.float32)
    for b in range(_NBLK):
        out += _dot(lhs[b * _H:(b + 1) * _H], w_ref[b * _ROWS:(b + 1) * _ROWS, :])
    return out


def _per_head_out(q, scale, e_ref, w_ref):
    full = jnp.concatenate(
        [_dot_nt(q, w_ref[b * _ROWS:(b + 1) * _ROWS, :]) for b in range(_NBLK)],
        axis=0)
    diag = jnp.where(_head_diag_mask(), full * scale, 0.0).astype(jnp.bfloat16)
    stack = _dot_nt(diag, e_ref[...]).astype(jnp.bfloat16)
    return jnp.concatenate(
        [stack[b * _H:(b + 1) * _H] for b in range(_NBLK)], axis=1)


def _kernel(x_hbm, ckv_hbm, wq_hbm, wuk_hbm, wuv_hbm, wo_hbm, wg_hbm, wu_hbm,
            wd_hbm, c_hbm, wmod_hbm, o_ref,
            x_v, c_v, wmod_v, wq_v, wuk_v, ckv_v, wuv_v, wo_v, wg_v,
            wu_v, e_v, y_v, acol_v, sems, *wd_v):

    def kv_copy(i):
        rows = pl.ds(_KV_SPLITS[i] * _T, (_KV_SPLITS[i + 1] - _KV_SPLITS[i]) * _T)
        return pltpu.make_async_copy(ckv_hbm.at[rows, :], ckv_v.at[rows, :],
                                     sems.at[6 + i])

    def wd_copy(i):
        rows = pl.ds(_WD_SPLITS[i], _WD_SPLITS[i + 1] - _WD_SPLITS[i])
        return pltpu.make_async_copy(wd_hbm.at[rows, :], wd_v[i],
                                     sems.at[6 + _NKV + i])

    cp_mod = pltpu.make_async_copy(wmod_hbm, wmod_v, sems.at[0])
    cp_c = pltpu.make_async_copy(c_hbm, c_v, sems.at[0])
    cp_x = pltpu.make_async_copy(x_hbm, x_v, sems.at[0])
    cp_wq = pltpu.make_async_copy(wq_hbm, wq_v, sems.at[1])
    cp_wuk = pltpu.make_async_copy(wuk_hbm, wuk_v, sems.at[2])
    cp_wuv = pltpu.make_async_copy(wuv_hbm, wuv_v, sems.at[3])
    cp_wo = pltpu.make_async_copy(wo_hbm, wo_v, sems.at[4])
    cp_wg = pltpu.make_async_copy(wg_hbm, wg_v, sems.at[5])
    cp_wu = pltpu.make_async_copy(wu_hbm, wu_v, sems.at[5])

    cp_mod.start()
    cp_c.start()
    cp_x.start()
    cp_wq.start()
    cp_wuk.start()
    for i in range(_NKV):
        kv_copy(i).start()
    cp_wuv.start()
    cp_wo.start()
    cp_wg.start()
    cp_wu.start()
    for i in range(len(_WD_SPLITS) - 1):
        wd_copy(i).start()

    with _scope("mk_e"):
        er = lax.broadcasted_iota(jnp.int32, (_BLK, _ROWS), 0)
        ec = lax.broadcasted_iota(jnp.int32, (_BLK, _ROWS), 1)
        e_v[...] = jnp.where(er == ec // _H, 1.0, 0.0).astype(jnp.bfloat16)

    with _scope("w_mod"):
        cp_c.wait()
        cp_x.wait()
        cp_mod.wait()
    with _scope("c_mod"):
        cf = c_v[...].astype(jnp.float32)
        sc = (cf * jax.nn.sigmoid(cf)).astype(jnp.bfloat16)
        mod_a = _dot(sc, wmod_v[:, :2 * _M])
        x = x_v[...].astype(jnp.float32)
        h = _layernorm(x) * (1.0 + mod_a[:, _M:]) + mod_a[:, :_M]
        h = jnp.broadcast_to(h, (_H, _M)).astype(jnp.bfloat16)
        mod_b = _dot(sc, wmod_v[:, 2 * _M:])

    with _scope("w_q"):
        cp_wq.wait()
    with _scope("c_q"):
        q = _per_head_in(h, e_v, wq_v).astype(jnp.bfloat16)
    with _scope("w_uk"):
        cp_wuk.wait()
    with _scope("c_uk"):
        q_abs = _per_head_out(q, _D ** -0.5, e_v, wuk_v)

    def kv_step(i, carry):
        m, l, acc = carry
        with _scope("w_kv"):
            for j in range(_NKV):
                pl.when(i == _KV_SPLITS[j])(kv_copy(j).wait)
        with _scope("c_kv"):
            ckv = ckv_v[pl.ds(pl.multiple_of(i * _T, _T), _T), :]
            s = _dot_nt(q_abs, ckv)
            m_new = jnp.maximum(m, jnp.max(s, axis=1, keepdims=True))
            alpha = jnp.exp(m - m_new)
            p = jnp.exp(s - m_new)
            l = alpha * l + jnp.sum(p, axis=1, keepdims=True)
            acc = alpha * acc + _dot(p.astype(jnp.bfloat16), ckv)
        return m_new, l, acc

    _, l, acc = lax.fori_loop(
        0, _NCHUNK, kv_step,
        (jnp.full((_H, 1), -jnp.inf, jnp.float32),
         jnp.zeros((_H, 1), jnp.float32),
         jnp.zeros((_H, _M), jnp.float32)))
    ctx_c = (acc / l).astype(jnp.bfloat16)

    with _scope("w_uv"):
        cp_wuv.wait()
    with _scope("c_uv"):
        ctx = _per_head_in(ctx_c, e_v, wuv_v)
        hr = lax.broadcasted_iota(jnp.int32, (_H, _H * _D), 0)
        hc = lax.broadcasted_iota(jnp.int32, (_H, _H * _D), 1)
        lhs = jnp.where(hr == hc // _D, jnp.concatenate([ctx] * _H, axis=1), 0.0)
        lhs = lhs.astype(jnp.bfloat16)
    with _scope("w_o"):
        cp_wo.wait()
    with _scope("c_o"):
        attn = jnp.sum(_dot(lhs, wo_v[...]), axis=0, keepdims=True)
        x1 = x + mod_b[:, :_M] * attn
        h2 = _layernorm(x1) * (1.0 + mod_b[:, 2 * _M:3 * _M]) + mod_b[:, _M:2 * _M]
        h2 = h2.astype(jnp.bfloat16)

    with _scope("w_g"):
        cp_wg.wait()
        cp_wu.wait()
    with _scope("c_g"):
        g = _gelu_tanh(_dot(h2, wg_v[...]))
    with _scope("c_u"):
        act = (g * _dot(h2, wu_v[...])).astype(jnp.bfloat16)
    n_wd = len(_WD_SPLITS) - 1
    with _scope("c_acol"):
        lo = _WD_SPLITS[-2]
        a_last = act[:, lo:].astype(jnp.float32)
        acol_v[...] = jnp.broadcast_to(a_last, (128, _F - lo)).T
    for i in range(n_wd - 1):
        lo, hi = _WD_SPLITS[i], _WD_SPLITS[i + 1]
        with _scope("w_d%d" % i):
            wd_copy(i).wait()
        with _scope("c_d%d" % i):
            part = _dot(act[:, lo:hi], wd_v[i][...])
            if i == 0:
                y_v[...] = part
            elif i < n_wd - 2:
                y_v[...] += part
    gb = mod_b[:, 3 * _M:]
    y_v[...] = x1 + gb * (y_v[...] + part)
    with _scope("w_dl"):
        wd_copy(n_wd - 1).wait()
    with _scope("c_dl"):
        acol = acol_v[...]
        cols = []
        for n in range(_M // 128):
            w = wd_v[-1][:, n * 128:(n + 1) * 128].astype(jnp.float32)
            cols.append(jnp.sum(w * acol, axis=0, keepdims=True))
        y_last = jnp.concatenate(cols, axis=1)
        o_ref[...] = (y_v[...] + gb * y_last).astype(o_ref.dtype)


@jax.jit
def pallas_adaLN_cond__compressed_kv_cla__glu_gated_geglu__decode_kernel(
A_x: jax.Array,
    A_c_kv: jax.Array,
    A_w_q: jax.Array,
    A_w_uk: jax.Array,
    A_w_uv: jax.Array,
    A_w_o: jax.Array,
    B_x: jax.Array,
    B_w_gate: jax.Array,
    B_w_up: jax.Array,
    B_w_down: jax.Array,
    c: jax.Array,
    w_mod: jax.Array,
):
    del B_x
    bf16 = jnp.bfloat16
    any_spec = pl.BlockSpec(memory_space=pl.ANY)
    out = pl.pallas_call(
        _kernel,
        in_specs=[any_spec] * 11,
        out_specs=pl.BlockSpec(memory_space=pltpu.VMEM),
        out_shape=jax.ShapeDtypeStruct((1, _M), A_x.dtype),
        scratch_shapes=[
            pltpu.VMEM((1, _M), bf16),
            pltpu.VMEM((1, _M), bf16),
            pltpu.VMEM((_M, 6 * _M), bf16),
            pltpu.VMEM((_M * _H, _D), bf16),
            pltpu.VMEM((_M * _H, _D), bf16),
            pltpu.VMEM((_SK, _M), bf16),
            pltpu.VMEM((_M * _H, _D), bf16),
            pltpu.VMEM((_H * _D, _M), bf16),
            pltpu.VMEM((_M, _F), bf16),
            pltpu.VMEM((_M, _F), bf16),
            pltpu.VMEM((_BLK, _ROWS), bf16),
            pltpu.VMEM((1, _M), jnp.float32),
            pltpu.VMEM((_F - _WD_SPLITS[-2], 128), jnp.float32),
            pltpu.SemaphoreType.DMA((6 + _NKV + len(_WD_SPLITS) - 1,)),
        ] + [pltpu.VMEM((hi - lo, _M), bf16)
             for lo, hi in zip(_WD_SPLITS[:-1], _WD_SPLITS[1:])],
        compiler_params=pltpu.CompilerParams(vmem_limit_bytes=100 * 1024 * 1024),
    )(
        A_x.reshape(1, _M),
        A_c_kv.reshape(_SK, _M),
        A_w_q.reshape(_M * _H, _D),
        A_w_uk.reshape(_M * _H, _D),
        A_w_uv.reshape(_M * _H, _D),
        A_w_o.reshape(_H * _D, _M),
        B_w_gate,
        B_w_up,
        B_w_down,
        c,
        w_mod,
    )
    return out.reshape(1, 1, _M)
```

```python
import functools

import jax
import jax.numpy as jnp
from jax import lax
import jax.experimental.pallas as pl
import jax.experimental.pallas.tpu as pltpu

_H = 32
_D = 128
_M = 512
_F = 1792
_SK = 32768
_T = 4096
_NCHUNK = _SK // _T
_BLK = 128
_ROWS = _BLK * _H
_NBLK = _M // _BLK
_KV_SPLITS = (0, 5, 8)
_NKV = len(_KV_SPLITS) - 1
_WD_SPLITS = (0, 1280, 1664, 1792)
_NWD = len(_WD_SPLITS) - 1
_EPS = 1e-5
_NT = (((1,), (1,)), ((), ()))


def _layernorm(x):
    mean = jnp.mean(x, axis=-1, keepdims=True)
    xc = x - mean
    var = jnp.mean(xc * xc, axis=-1, keepdims=True)
    return xc / jnp.sqrt(var + _EPS)


def _gelu_tanh(x):
    k = 0.7978845608028654
    return 0.5 * x * (1.0 + jnp.tanh(k * (x + 0.044715 * (x * x * x))))


def _dot(a, b):
    return jnp.dot(a, b, preferred_element_type=jnp.float32)


def _dot_nt(a, b):
    return lax.dot_general(a, b, _NT, preferred_element_type=jnp.float32)


def _head_diag_mask():
    r = lax.broadcasted_iota(jnp.int32, (_NBLK * _H, _ROWS), 0)
    c = lax.broadcasted_iota(jnp.int32, (_NBLK * _H, _ROWS), 1)
    return (r % _H) == (c % _H)


def _per_head_in(a, e_ref, w_ref):
    a_stack = jnp.concatenate(
        [a[:, b * _BLK:(b + 1) * _BLK] for b in range(_NBLK)], axis=0)
    y = _dot(a_stack, e_ref[...])
    lhs = jnp.where(_head_diag_mask(), y, 0.0).astype(jnp.bfloat16)
    out = jnp.zeros((_H, _D), jnp.float32)
    for b in range(_NBLK):
        out += _dot(lhs[b * _H:(b + 1) * _H], w_ref[b * _ROWS:(b + 1) * _ROWS, :])
    return out


def _per_head_out(q, scale, e_ref, w_ref):
    full = jnp.concatenate(
        [_dot_nt(q, w_ref[b * _ROWS:(b + 1) * _ROWS, :]) for b in range(_NBLK)],
        axis=0)
    diag = jnp.where(_head_diag_mask(), full * scale, 0.0).astype(jnp.bfloat16)
    stack = _dot_nt(diag, e_ref[...]).astype(jnp.bfloat16)
    return jnp.concatenate(
        [stack[b * _H:(b + 1) * _H] for b in range(_NBLK)], axis=1)


def _kernel(x_hbm, ckv_hbm, wq_hbm, wuk_hbm, wuv_hbm, wo_hbm, wg_hbm, wu_hbm,
            wd_hbm, c_hbm, wmod_hbm, o_ref, *scratch):
    pl.run_scoped(
        functools.partial(
            _body, (x_hbm, ckv_hbm, wq_hbm, wuk_hbm, wuv_hbm, wo_hbm, wg_hbm,
                    wu_hbm, wd_hbm, c_hbm, wmod_hbm), o_ref, scratch),
        pltpu.SemaphoreType.DMA((9 + _NKV + _NWD,)))


def _body(hbm, o_ref, scratch, sems):
    (x_hbm, ckv_hbm, wq_hbm, wuk_hbm, wuv_hbm, wo_hbm, wg_hbm, wu_hbm, wd_hbm,
     c_hbm, wmod_hbm) = hbm
    (x_v, c_v, wmod_v, wq_v, wuk_v, ckv_v, wuv_v, wo_v, wg_v, wu_v, e_v, y_v,
     acol_v, *wd_v) = scratch

    def copy(src, dst, i):
        return pltpu.make_async_copy(src, dst, sems.at[i])

    def kv_copy(i):
        rows = pl.ds(_KV_SPLITS[i] * _T, (_KV_SPLITS[i + 1] - _KV_SPLITS[i]) * _T)
        return copy(ckv_hbm.at[rows, :], ckv_v.at[rows, :], 9 + i)

    def wd_copy(i):
        rows = pl.ds(_WD_SPLITS[i], _WD_SPLITS[i + 1] - _WD_SPLITS[i])
        return copy(wd_hbm.at[rows, :], wd_v[i], 9 + _NKV + i)

    cp_mod, cp_c, cp_x = copy(wmod_hbm, wmod_v, 0), copy(c_hbm, c_v, 1), copy(x_hbm, x_v, 2)
    cp_wq, cp_wuk = copy(wq_hbm, wq_v, 3), copy(wuk_hbm, wuk_v, 4)
    cp_wuv, cp_wo = copy(wuv_hbm, wuv_v, 5), copy(wo_hbm, wo_v, 6)
    cp_wg, cp_wu = copy(wg_hbm, wg_v, 7), copy(wu_hbm, wu_v, 8)
    for cp in (cp_mod, cp_c, cp_x, cp_wq, cp_wuk,
               *[kv_copy(i) for i in range(_NKV)],
               cp_wuv, cp_wo, cp_wg, cp_wu,
               *[wd_copy(i) for i in range(_NWD)]):
        cp.start()

    er = lax.broadcasted_iota(jnp.int32, (_BLK, _ROWS), 0)
    ec = lax.broadcasted_iota(jnp.int32, (_BLK, _ROWS), 1)
    e_v[...] = jnp.where(er == ec // _H, 1.0, 0.0).astype(jnp.bfloat16)

    cp_c.wait()
    cp_x.wait()
    cp_mod.wait()
    cf = c_v[...].astype(jnp.float32)
    sc = (cf * jax.nn.sigmoid(cf)).astype(jnp.bfloat16)
    mod_a = _dot(sc, wmod_v[:, :2 * _M])
    x = x_v[...].astype(jnp.float32)
    h = _layernorm(x) * (1.0 + mod_a[:, _M:]) + mod_a[:, :_M]
    h = jnp.broadcast_to(h, (_H, _M)).astype(jnp.bfloat16)
    mod_b = _dot(sc, wmod_v[:, 2 * _M:])

    cp_wq.wait()
    q = _per_head_in(h, e_v, wq_v).astype(jnp.bfloat16)
    cp_wuk.wait()
    q_abs = _per_head_out(q, _D ** -0.5, e_v, wuk_v)

    def kv_step(i, carry):
        m, l, acc = carry
        for j in range(_NKV):
            pl.when(i == _KV_SPLITS[j])(kv_copy(j).wait)
        ckv = ckv_v[pl.ds(pl.multiple_of(i * _T, _T), _T), :]
        s = _dot_nt(q_abs, ckv)
        m_new = jnp.maximum(m, jnp.max(s, axis=1, keepdims=True))
        alpha = jnp.exp(m - m_new)
        p = jnp.exp(s - m_new)
        l = alpha * l + jnp.sum(p, axis=1, keepdims=True)
        acc = alpha * acc + _dot(p.astype(jnp.bfloat16), ckv)
        return m_new, l, acc

    _, l, acc = lax.fori_loop(
        0, _NCHUNK, kv_step,
        (jnp.full((_H, 1), -jnp.inf, jnp.float32),
         jnp.zeros((_H, 1), jnp.float32),
         jnp.zeros((_H, _M), jnp.float32)))
    ctx_c = (acc / l).astype(jnp.bfloat16)

    cp_wuv.wait()
    ctx = _per_head_in(ctx_c, e_v, wuv_v)
    hr = lax.broadcasted_iota(jnp.int32, (_H, _H * _D), 0)
    hc = lax.broadcasted_iota(jnp.int32, (_H, _H * _D), 1)
    lhs = jnp.where(hr == hc // _D, jnp.concatenate([ctx] * _H, axis=1), 0.0)
    lhs = lhs.astype(jnp.bfloat16)
    cp_wo.wait()
    attn = jnp.sum(_dot(lhs, wo_v[...]), axis=0, keepdims=True)

    x1 = x + mod_b[:, :_M] * attn
    h2 = _layernorm(x1) * (1.0 + mod_b[:, 2 * _M:3 * _M]) + mod_b[:, _M:2 * _M]
    h2 = h2.astype(jnp.bfloat16)
    cp_wg.wait()
    g = _gelu_tanh(_dot(h2, wg_v[...]))
    cp_wu.wait()
    act = (g * _dot(h2, wu_v[...])).astype(jnp.bfloat16)

    lo = _WD_SPLITS[-2]
    acol_v[...] = jnp.broadcast_to(act[:, lo:].astype(jnp.float32), (128, _F - lo)).T
    for i in range(_NWD - 1):
        lo, hi = _WD_SPLITS[i], _WD_SPLITS[i + 1]
        wd_copy(i).wait()
        part = _dot(act[:, lo:hi], wd_v[i][...])
        if i == 0:
            y_v[...] = part
        elif i < _NWD - 2:
            y_v[...] += part
    gb = mod_b[:, 3 * _M:]
    y_v[...] = x1 + gb * (y_v[...] + part)
    wd_copy(_NWD - 1).wait()
    acol = acol_v[...]
    cols = []
    for n in range(_M // 128):
        w = wd_v[-1][:, n * 128:(n + 1) * 128].astype(jnp.float32)
        cols.append(jnp.sum(w * acol, axis=0, keepdims=True))
    y_last = jnp.concatenate(cols, axis=1)
    o_ref[...] = (y_v[...] + gb * y_last).astype(o_ref.dtype)


@jax.jit
def pallas_adaLN_cond__compressed_kv_cla__glu_gated_geglu__decode_kernel(
A_x: jax.Array,
    A_c_kv: jax.Array,
    A_w_q: jax.Array,
    A_w_uk: jax.Array,
    A_w_uv: jax.Array,
    A_w_o: jax.Array,
    B_x: jax.Array,
    B_w_gate: jax.Array,
    B_w_up: jax.Array,
    B_w_down: jax.Array,
    c: jax.Array,
    w_mod: jax.Array,
):
    del B_x
    bf16 = jnp.bfloat16
    any_spec = pl.BlockSpec(memory_space=pl.ANY)
    out = pl.pallas_call(
        _kernel,
        in_specs=[any_spec] * 11,
        out_specs=pl.BlockSpec(memory_space=pltpu.VMEM),
        out_shape=jax.ShapeDtypeStruct((1, _M), A_x.dtype),
        scratch_shapes=[
            pltpu.VMEM((1, _M), bf16),
            pltpu.VMEM((1, _M), bf16),
            pltpu.VMEM((_M, 6 * _M), bf16),
            pltpu.VMEM((_M * _H, _D), bf16),
            pltpu.VMEM((_M * _H, _D), bf16),
            pltpu.VMEM((_SK, _M), bf16),
            pltpu.VMEM((_M * _H, _D), bf16),
            pltpu.VMEM((_H * _D, _M), bf16),
            pltpu.VMEM((_M, _F), bf16),
            pltpu.VMEM((_M, _F), bf16),
            pltpu.VMEM((_BLK, _ROWS), bf16),
            pltpu.VMEM((1, _M), jnp.float32),
            pltpu.VMEM((_F - _WD_SPLITS[-2], 128), jnp.float32),
        ] + [pltpu.VMEM((hi - lo, _M), bf16)
             for lo, hi in zip(_WD_SPLITS[:-1], _WD_SPLITS[1:])],
        compiler_params=pltpu.CompilerParams(vmem_limit_bytes=100 * 1024 * 1024),
    )(
        A_x.reshape(1, _M),
        A_c_kv.reshape(_SK, _M),
        A_w_q.reshape(_M * _H, _D),
        A_w_uk.reshape(_M * _H, _D),
        A_w_uv.reshape(_M * _H, _D),
        A_w_o.reshape(_H * _D, _M),
        B_w_gate,
        B_w_up,
        B_w_down,
        c,
        w_mod,
    )
    return out.reshape(1, 1, _M)
```

```python
import functools

import jax
import jax.numpy as jnp
from jax import lax
import jax.experimental.pallas as pl
import jax.experimental.pallas.tpu as pltpu

_H = 32
_D = 128
_M = 512
_F = 1792
_SK = 32768
_T = 4096
_NCHUNK = _SK // _T
_BLK = 128
_ROWS = _BLK * _H
_NBLK = _M // _BLK
_KV_SPLITS = (0, 5, 8)
_NKV = len(_KV_SPLITS) - 1
_WD_SPLITS = (0, 1280, 1536, 1664, 1744, 1776, 1792)
_NWD_MXU = 2
_NWD = len(_WD_SPLITS) - 1
_EPS = 1e-5
_NT = (((1,), (1,)), ((), ()))


def _layernorm(x):
    mean = jnp.mean(x, axis=-1, keepdims=True)
    xc = x - mean
    var = jnp.mean(xc * xc, axis=-1, keepdims=True)
    return xc / jnp.sqrt(var + _EPS)


def _gelu_tanh(x):
    k = 0.7978845608028654
    return 0.5 * x * (1.0 + jnp.tanh(k * (x + 0.044715 * (x * x * x))))


def _dot(a, b):
    return jnp.dot(a, b, preferred_element_type=jnp.float32)


def _dot_nt(a, b):
    return lax.dot_general(a, b, _NT, preferred_element_type=jnp.float32)


def _head_diag_mask():
    r = lax.broadcasted_iota(jnp.int32, (_NBLK * _H, _ROWS), 0)
    c = lax.broadcasted_iota(jnp.int32, (_NBLK * _H, _ROWS), 1)
    return (r % _H) == (c % _H)


def _per_head_in(a, e_ref, w_ref):
    a_stack = jnp.concatenate(
        [a[:, b * _BLK:(b + 1) * _BLK] for b in range(_NBLK)], axis=0)
    y = _dot(a_stack, e_ref[...])
    lhs = jnp.where(_head_diag_mask(), y, 0.0).astype(jnp.bfloat16)
    out = jnp.zeros((_H, _D), jnp.float32)
    for b in range(_NBLK):
        out += _dot(lhs[b * _H:(b + 1) * _H], w_ref[b * _ROWS:(b + 1) * _ROWS, :])
    return out


def _per_head_out(q, scale, e_ref, w_ref):
    full = jnp.concatenate(
        [_dot_nt(q, w_ref[b * _ROWS:(b + 1) * _ROWS, :]) for b in range(_NBLK)],
        axis=0)
    diag = jnp.where(_head_diag_mask(), full * scale, 0.0).astype(jnp.bfloat16)
    stack = _dot_nt(diag, e_ref[...]).astype(jnp.bfloat16)
    return jnp.concatenate(
        [stack[b * _H:(b + 1) * _H] for b in range(_NBLK)], axis=1)


def _kernel(x_hbm, ckv_hbm, wq_hbm, wuk_hbm, wuv_hbm, wo_hbm, wg_hbm, wu_hbm,
            wd_hbm, c_hbm, wmod_hbm, o_ref, *scratch):
    pl.run_scoped(
        functools.partial(
            _body, (x_hbm, ckv_hbm, wq_hbm, wuk_hbm, wuv_hbm, wo_hbm, wg_hbm,
                    wu_hbm, wd_hbm, c_hbm, wmod_hbm), o_ref, scratch),
        pltpu.SemaphoreType.DMA((9 + _NKV + _NWD,)))


def _body(hbm, o_ref, scratch, sems):
    (x_hbm, ckv_hbm, wq_hbm, wuk_hbm, wuv_hbm, wo_hbm, wg_hbm, wu_hbm, wd_hbm,
     c_hbm, wmod_hbm) = hbm
    (x_v, c_v, wmod_v, wq_v, wuk_v, ckv_v, wuv_v, wo_v, wg_v, wu_v, e_v, y_v,
     acol_v, *wd_v) = scratch

    def copy(src, dst, i):
        return pltpu.make_async_copy(src, dst, sems.at[i])

    def kv_copy(i):
        rows = pl.ds(_KV_SPLITS[i] * _T, (_KV_SPLITS[i + 1] - _KV_SPLITS[i]) * _T)
        return copy(ckv_hbm.at[rows, :], ckv_v.at[rows, :], 9 + i)

    def wd_copy(i):
        rows = pl.ds(_WD_SPLITS[i], _WD_SPLITS[i + 1] - _WD_SPLITS[i])
        return copy(wd_hbm.at[rows, :], wd_v[i], 9 + _NKV + i)

    cp_mod, cp_c, cp_x = copy(wmod_hbm, wmod_v, 0), copy(c_hbm, c_v, 1), copy(x_hbm, x_v, 2)
    cp_wq, cp_wuk = copy(wq_hbm, wq_v, 3), copy(wuk_hbm, wuk_v, 4)
    cp_wuv, cp_wo = copy(wuv_hbm, wuv_v, 5), copy(wo_hbm, wo_v, 6)
    cp_wg, cp_wu = copy(wg_hbm, wg_v, 7), copy(wu_hbm, wu_v, 8)
    for cp in (cp_mod, cp_c, cp_x, cp_wq, cp_wuk,
               *[kv_copy(i) for i in range(_NKV)],
               cp_wuv, cp_wo, cp_wg, cp_wu,
               *[wd_copy(i) for i in range(_NWD)]):
        cp.start()

    er = lax.broadcasted_iota(jnp.int32, (_BLK, _ROWS), 0)
    ec = lax.broadcasted_iota(jnp.int32, (_BLK, _ROWS), 1)
    e_v[...] = jnp.where(er == ec // _H, 1.0, 0.0).astype(jnp.bfloat16)

    cp_c.wait()
    cp_x.wait()
    cp_mod.wait()
    cf = c_v[...].astype(jnp.float32)
    sc = (cf * jax.nn.sigmoid(cf)).astype(jnp.bfloat16)
    mod_a = _dot(sc, wmod_v[:, :2 * _M])
    x = x_v[...].astype(jnp.float32)
    h = _layernorm(x) * (1.0 + mod_a[:, _M:]) + mod_a[:, :_M]
    h = jnp.broadcast_to(h, (_H, _M)).astype(jnp.bfloat16)
    mod_b = _dot(sc, wmod_v[:, 2 * _M:])

    cp_wq.wait()
    q = _per_head_in(h, e_v, wq_v).astype(jnp.bfloat16)
    cp_wuk.wait()
    q_abs = _per_head_out(q, _D ** -0.5, e_v, wuk_v)

    def kv_step(i, carry):
        m, l, acc = carry
        for j in range(_NKV):
            pl.when(i == _KV_SPLITS[j])(kv_copy(j).wait)
        ckv = ckv_v[pl.ds(pl.multiple_of(i * _T, _T), _T), :]
        s = _dot_nt(q_abs, ckv)
        m_new = jnp.maximum(m, jnp.max(s, axis=1, keepdims=True))
        alpha = jnp.exp(m - m_new)
        p = jnp.exp(s - m_new)
        l = alpha * l + jnp.sum(p, axis=1, keepdims=True)
        acc = alpha * acc + _dot(p.astype(jnp.bfloat16), ckv)
        return m_new, l, acc

    _, l, acc = lax.fori_loop(
        0, _NCHUNK, kv_step,
        (jnp.full((_H, 1), -jnp.inf, jnp.float32),
         jnp.zeros((_H, 1), jnp.float32),
         jnp.zeros((_H, _M), jnp.float32)))
    ctx_c = (acc / l).astype(jnp.bfloat16)

    cp_wuv.wait()
    ctx = _per_head_in(ctx_c, e_v, wuv_v)
    hr = lax.broadcasted_iota(jnp.int32, (_H, _H * _D), 0)
    hc = lax.broadcasted_iota(jnp.int32, (_H, _H * _D), 1)
    lhs = jnp.where(hr == hc // _D, jnp.concatenate([ctx] * _H, axis=1), 0.0)
    lhs = lhs.astype(jnp.bfloat16)
    cp_wo.wait()
    attn = jnp.sum(_dot(lhs, wo_v[...]), axis=0, keepdims=True)

    x1 = x + mod_b[:, :_M] * attn
    h2 = _layernorm(x1) * (1.0 + mod_b[:, 2 * _M:3 * _M]) + mod_b[:, _M:2 * _M]
    h2 = h2.astype(jnp.bfloat16)
    cp_wg.wait()
    g = _gelu_tanh(_dot(h2, wg_v[...]))
    cp_wu.wait()
    act = (g * _dot(h2, wu_v[...])).astype(jnp.bfloat16)

    v0 = _WD_SPLITS[_NWD_MXU]
    for r in range(v0, _F, 128):
        acol_v[r - v0:r - v0 + 128, :] = jnp.broadcast_to(
            act[:, r:r + 128].astype(jnp.float32), (128, 128)).T
    for i in range(_NWD_MXU):
        lo, hi = _WD_SPLITS[i], _WD_SPLITS[i + 1]
        wd_copy(i).wait()
        part = _dot(act[:, lo:hi], wd_v[i][...])
        if i == 0:
            y_v[...] = part
        elif i < _NWD_MXU - 1:
            y_v[...] += part
    gb = mod_b[:, 3 * _M:]
    y_v[...] = x1 + gb * (y_v[...] + part)
    accs = [None] * (_M // 128)
    for i in range(_NWD_MXU, _NWD):
        lo, hi = _WD_SPLITS[i], _WD_SPLITS[i + 1]
        wd_copy(i).wait()
        acol = acol_v[lo - v0:hi - v0, :]
        for n in range(_M // 128):
            w = wd_v[i][:, n * 128:(n + 1) * 128].astype(jnp.float32)
            part = jnp.sum((w * acol).reshape((hi - lo) // 8, 8, 128), axis=0)
            accs[n] = part if accs[n] is None else accs[n] + part
    y_last = jnp.concatenate([jnp.sum(a, axis=0, keepdims=True) for a in accs], axis=1)
    o_ref[...] = (y_v[...] + gb * y_last).astype(o_ref.dtype)


@jax.jit
def pallas_adaLN_cond__compressed_kv_cla__glu_gated_geglu__decode_kernel(
A_x: jax.Array,
    A_c_kv: jax.Array,
    A_w_q: jax.Array,
    A_w_uk: jax.Array,
    A_w_uv: jax.Array,
    A_w_o: jax.Array,
    B_x: jax.Array,
    B_w_gate: jax.Array,
    B_w_up: jax.Array,
    B_w_down: jax.Array,
    c: jax.Array,
    w_mod: jax.Array,
):
    del B_x
    bf16 = jnp.bfloat16
    any_spec = pl.BlockSpec(memory_space=pl.ANY)
    out = pl.pallas_call(
        _kernel,
        in_specs=[any_spec] * 11,
        out_specs=pl.BlockSpec(memory_space=pltpu.VMEM),
        out_shape=jax.ShapeDtypeStruct((1, _M), A_x.dtype),
        scratch_shapes=[
            pltpu.VMEM((1, _M), bf16),
            pltpu.VMEM((1, _M), bf16),
            pltpu.VMEM((_M, 6 * _M), bf16),
            pltpu.VMEM((_M * _H, _D), bf16),
            pltpu.VMEM((_M * _H, _D), bf16),
            pltpu.VMEM((_SK, _M), bf16),
            pltpu.VMEM((_M * _H, _D), bf16),
            pltpu.VMEM((_H * _D, _M), bf16),
            pltpu.VMEM((_M, _F), bf16),
            pltpu.VMEM((_M, _F), bf16),
            pltpu.VMEM((_BLK, _ROWS), bf16),
            pltpu.VMEM((1, _M), jnp.float32),
            pltpu.VMEM((_F - _WD_SPLITS[_NWD_MXU], 128), jnp.float32),
        ] + [pltpu.VMEM((hi - lo, _M), bf16)
             for lo, hi in zip(_WD_SPLITS[:-1], _WD_SPLITS[1:])],
        compiler_params=pltpu.CompilerParams(vmem_limit_bytes=100 * 1024 * 1024),
    )(
        A_x.reshape(1, _M),
        A_c_kv.reshape(_SK, _M),
        A_w_q.reshape(_M * _H, _D),
        A_w_uk.reshape(_M * _H, _D),
        A_w_uv.reshape(_M * _H, _D),
        A_w_o.reshape(_H * _D, _M),
        B_w_gate,
        B_w_up,
        B_w_down,
        c,
        w_mod,
    )
    return out.reshape(1, 1, _M)
```

```python
import functools

import jax
import jax.numpy as jnp
from jax import lax
import jax.experimental.pallas as pl
import jax.experimental.pallas.tpu as pltpu

_H = 32
_D = 128
_M = 512
_F = 1792
_SK = 32768
_T = 4096
_NCHUNK = _SK // _T
_BLK = 128
_ROWS = _BLK * _H
_NBLK = _M // _BLK
_WD_SPLITS = (0, 1280, 1536, 1664, 1744, 1776, 1792)
_NWD = len(_WD_SPLITS) - 1
_NWD_MXU = 2
_NS = 9
_EPS = 1e-5
_NT = (((1,), (1,)), ((), ()))


def _layernorm(x):
    mean = jnp.mean(x, axis=-1, keepdims=True)
    xc = x - mean
    var = jnp.mean(xc * xc, axis=-1, keepdims=True)
    return xc / jnp.sqrt(var + _EPS)


def _gelu_tanh(x):
    k = 0.7978845608028654
    return 0.5 * x * (1.0 + jnp.tanh(k * (x + 0.044715 * (x * x * x))))


def _dot(a, b):
    return jnp.dot(a, b, preferred_element_type=jnp.float32)


def _dot_nt(a, b):
    return lax.dot_general(a, b, _NT, preferred_element_type=jnp.float32)


def _head_diag_mask():
    r = lax.broadcasted_iota(jnp.int32, (_NBLK * _H, _ROWS), 0)
    c = lax.broadcasted_iota(jnp.int32, (_NBLK * _H, _ROWS), 1)
    return (r % _H) == (c % _H)


def _per_head_in(a, e_ref, w_ref):
    a_stack = jnp.concatenate(
        [a[:, b * _BLK:(b + 1) * _BLK] for b in range(_NBLK)], axis=0)
    spread = _dot(a_stack, e_ref[...])
    lhs = jnp.where(_head_diag_mask(), spread, 0.0).astype(jnp.bfloat16)
    out = jnp.zeros((_H, _D), jnp.float32)
    for b in range(_NBLK):
        out += _dot(lhs[b * _H:(b + 1) * _H], w_ref[b * _ROWS:(b + 1) * _ROWS, :])
    return out


def _per_head_out(q, scale, e_ref, w_ref):
    full = jnp.concatenate(
        [_dot_nt(q, w_ref[b * _ROWS:(b + 1) * _ROWS, :]) for b in range(_NBLK)],
        axis=0)
    diag = jnp.where(_head_diag_mask(), full * scale, 0.0).astype(jnp.bfloat16)
    stack = _dot_nt(diag, e_ref[...]).astype(jnp.bfloat16)
    return jnp.concatenate(
        [stack[b * _H:(b + 1) * _H] for b in range(_NBLK)], axis=1)


def _body(x_hbm, ckv_hbm, wq_hbm, wuk_hbm, wuv_hbm, wo_hbm, wg_hbm, wu_hbm,
          wd_hbm, c_hbm, wmod_hbm, o_ref,
          x_v, c_v, wmod_v, wq_v, wuk_v, ckv_v, wuv_v, wo_v, wg_v, wu_v,
          e_v, y_v, acol_v, wd_v, sems):

    def copy(src, dst, i):
        return pltpu.make_async_copy(src, dst, sems.at[i])

    def kv_copy(i):
        rows = pl.ds(pl.multiple_of(i * _T, _T), _T)
        return copy(ckv_hbm.at[rows, :], ckv_v.at[rows, :], _NS + i)

    def wd_copy(i):
        rows = pl.ds(_WD_SPLITS[i], _WD_SPLITS[i + 1] - _WD_SPLITS[i])
        return copy(wd_hbm.at[rows, :], wd_v[i], _NS + _NCHUNK + i)

    cp_mod, cp_c, cp_x = copy(wmod_hbm, wmod_v, 0), copy(c_hbm, c_v, 1), copy(x_hbm, x_v, 2)
    cp_wq, cp_wuk = copy(wq_hbm, wq_v, 3), copy(wuk_hbm, wuk_v, 4)
    cp_wuv, cp_wo = copy(wuv_hbm, wuv_v, 5), copy(wo_hbm, wo_v, 6)
    cp_wg, cp_wu = copy(wg_hbm, wg_v, 7), copy(wu_hbm, wu_v, 8)
    for cp in (cp_mod, cp_c, cp_x, cp_wq, cp_wuk,
               *[kv_copy(i) for i in range(_NCHUNK)],
               cp_wuv, cp_wo, cp_wg, cp_wu,
               *[wd_copy(i) for i in range(_NWD)]):
        cp.start()

    er = lax.broadcasted_iota(jnp.int32, (_BLK, _ROWS), 0)
    ec = lax.broadcasted_iota(jnp.int32, (_BLK, _ROWS), 1)
    e_v[...] = jnp.where(er == ec // _H, 1.0, 0.0).astype(jnp.bfloat16)

    cp_c.wait()
    cp_x.wait()
    cp_mod.wait()
    cf = c_v[...].astype(jnp.float32)
    sc = (cf * jax.nn.sigmoid(cf)).astype(jnp.bfloat16)
    mod_a = _dot(sc, wmod_v[:, :2 * _M])
    x = x_v[...].astype(jnp.float32)
    h = _layernorm(x) * (1.0 + mod_a[:, _M:]) + mod_a[:, :_M]
    h = jnp.broadcast_to(h, (_H, _M)).astype(jnp.bfloat16)
    mod_b = _dot(sc, wmod_v[:, 2 * _M:])

    cp_wq.wait()
    q = _per_head_in(h, e_v, wq_v).astype(jnp.bfloat16)
    cp_wuk.wait()
    q_abs = _per_head_out(q, _D ** -0.5, e_v, wuk_v)

    def kv_step(i, carry):
        m, l, acc = carry
        kv_copy(i).wait()
        ckv = ckv_v[pl.ds(pl.multiple_of(i * _T, _T), _T), :]
        s = _dot_nt(q_abs, ckv)
        m_new = jnp.maximum(m, jnp.max(s, axis=1, keepdims=True))
        alpha = jnp.exp(m - m_new)
        p = jnp.exp(s - m_new)
        l = alpha * l + jnp.sum(p, axis=1, keepdims=True)
        acc = alpha * acc + _dot(p.astype(jnp.bfloat16), ckv)
        return m_new, l, acc

    _, l, acc = lax.fori_loop(
        0, _NCHUNK, kv_step,
        (jnp.full((_H, 1), -jnp.inf, jnp.float32),
         jnp.zeros((_H, 1), jnp.float32),
         jnp.zeros((_H, _M), jnp.float32)))
    ctx_c = (acc / l).astype(jnp.bfloat16)

    cp_wuv.wait()
    ctx = _per_head_in(ctx_c, e_v, wuv_v)
    hr = lax.broadcasted_iota(jnp.int32, (_H, _H * _D), 0)
    hc = lax.broadcasted_iota(jnp.int32, (_H, _H * _D), 1)
    lhs = jnp.where(hr == hc // _D, jnp.concatenate([ctx] * _H, axis=1), 0.0)
    lhs = lhs.astype(jnp.bfloat16)
    cp_wo.wait()
    attn = jnp.sum(_dot(lhs, wo_v[...]), axis=0, keepdims=True)

    x1 = x + mod_b[:, :_M] * attn
    h2 = _layernorm(x1) * (1.0 + mod_b[:, 2 * _M:3 * _M]) + mod_b[:, _M:2 * _M]
    h2 = h2.astype(jnp.bfloat16)
    cp_wg.wait()
    g = _gelu_tanh(_dot(h2, wg_v[...]))
    cp_wu.wait()
    act = (g * _dot(h2, wu_v[...])).astype(jnp.bfloat16)

    v0 = _WD_SPLITS[_NWD_MXU]
    for r in range(v0, _F, 128):
        acol_v[r - v0:r - v0 + 128, :] = jnp.broadcast_to(
            act[:, r:r + 128].astype(jnp.float32), (128, 128)).T
    for i in range(_NWD_MXU):
        lo, hi = _WD_SPLITS[i], _WD_SPLITS[i + 1]
        wd_copy(i).wait()
        part = _dot(act[:, lo:hi], wd_v[i][...])
        if i == 0:
            y_v[...] = part
        elif i < _NWD_MXU - 1:
            y_v[...] += part
    gb = mod_b[:, 3 * _M:]
    y_v[...] = x1 + gb * (y_v[...] + part)
    accs = [None] * (_M // 128)
    for i in range(_NWD_MXU, _NWD):
        lo, hi = _WD_SPLITS[i], _WD_SPLITS[i + 1]
        wd_copy(i).wait()
        acol = acol_v[lo - v0:hi - v0, :]
        for n in range(_M // 128):
            w = wd_v[i][:, n * 128:(n + 1) * 128].astype(jnp.float32)
            part = jnp.sum((w * acol).reshape((hi - lo) // 8, 8, 128), axis=0)
            accs[n] = part if accs[n] is None else accs[n] + part
    y_last = jnp.concatenate(
        [jnp.sum(a, axis=0, keepdims=True) for a in accs], axis=1)
    o_ref[...] = (y_v[...] + gb * y_last).astype(o_ref.dtype)


def _kernel(*refs):
    n = len(refs) - _NWD
    pl.run_scoped(functools.partial(_body, *refs[:n], refs[n:]),
                  pltpu.SemaphoreType.DMA((_NS + _NCHUNK + _NWD,)))


@jax.jit
def pallas_adaLN_cond__compressed_kv_cla__glu_gated_geglu__decode_kernel(
A_x: jax.Array,
    A_c_kv: jax.Array,
    A_w_q: jax.Array,
    A_w_uk: jax.Array,
    A_w_uv: jax.Array,
    A_w_o: jax.Array,
    B_x: jax.Array,
    B_w_gate: jax.Array,
    B_w_up: jax.Array,
    B_w_down: jax.Array,
    c: jax.Array,
    w_mod: jax.Array,
):
    del B_x
    bf16 = jnp.bfloat16
    any_spec = pl.BlockSpec(memory_space=pl.ANY)
    out = pl.pallas_call(
        _kernel,
        in_specs=[any_spec] * 11,
        out_specs=pl.BlockSpec(memory_space=pltpu.VMEM),
        out_shape=jax.ShapeDtypeStruct((1, _M), A_x.dtype),
        scratch_shapes=[
            pltpu.VMEM((1, _M), bf16),
            pltpu.VMEM((1, _M), bf16),
            pltpu.VMEM((_M, 6 * _M), bf16),
            pltpu.VMEM((_M * _H, _D), bf16),
            pltpu.VMEM((_M * _H, _D), bf16),
            pltpu.VMEM((_SK, _M), bf16),
            pltpu.VMEM((_M * _H, _D), bf16),
            pltpu.VMEM((_H * _D, _M), bf16),
            pltpu.VMEM((_M, _F), bf16),
            pltpu.VMEM((_M, _F), bf16),
            pltpu.VMEM((_BLK, _ROWS), bf16),
            pltpu.VMEM((1, _M), jnp.float32),
            pltpu.VMEM((_F - _WD_SPLITS[_NWD_MXU], 128), jnp.float32),
        ] + [pltpu.VMEM((hi - lo, _M), bf16)
             for lo, hi in zip(_WD_SPLITS[:-1], _WD_SPLITS[1:])],
        compiler_params=pltpu.CompilerParams(vmem_limit_bytes=100 * 1024 * 1024),
    )(
        A_x.reshape(1, _M),
        A_c_kv.reshape(_SK, _M),
        A_w_q.reshape(_M * _H, _D),
        A_w_uk.reshape(_M * _H, _D),
        A_w_uv.reshape(_M * _H, _D),
        A_w_o.reshape(_H * _D, _M),
        B_w_gate,
        B_w_up,
        B_w_down,
        c,
        w_mod,
    )
    return out.reshape(1, 1, _M)
```
